```python
import jax
import jax.numpy as jnp

def _softmax(x, axis=-1):
    return jax.nn.softmax(x, axis=axis)
def _gelu(x):
    return jax.nn.gelu(x, approximate=True)
def _silu(x):
    return jax.nn.silu(x)
def _sigmoid(x):
    return jax.nn.sigmoid(x)
def _layernorm(x, axis=-1, eps=1e-5):
    m = jnp.mean(x, axis=axis, keepdims=True)
    v = jnp.var(x, axis=axis, keepdims=True)
    return (x - m) / jnp.sqrt(v + eps)
def _scatter_add(tgt, idx, src, axis=0):
    return tgt.at[idx].add(src)
def _segment_sum(src, seg, n):
    return jax.ops.segment_sum(src, seg, n)
class _Rng:
    def __init__(self, key):
        self._k = key
    def _next(self):
        self._k, sub = jax.random.split(self._k)
        return sub
    def normal(self, shape):
        return jax.random.normal(self._next(), shape, dtype=jnp.bfloat16)
    def randint(self, lo, hi, shape):
        return jax.random.randint(self._next(), shape, lo, hi, dtype=jnp.int32)
    def uniform(self, shape, lo=0.0, hi=1.0):
        return jax.random.uniform(self._next(), shape, jnp.bfloat16, lo, hi)
    def permutation(self, n):
        return jax.random.permutation(self._next(), n)


kernel_name = 'gated_mix__mha_block_cached__compressed_kv_cla__decode'

def setup_inputs():
    _rng = _Rng(jax.random.key(int.from_bytes(__import__("os").urandom(4), "little")))
    _w = (lambda a: (lambda t: t.astype(jnp.bfloat16) if jnp.issubdtype(t.dtype, jnp.floating) else t)(jnp.asarray(a)))
    def _A_setup():
        B, Sq, D = 2, 1, 512
        H, Sk, Dh = 32, 8192, 128
        return {
            "x": _w((lambda *s: _rng.normal(s) * 0.05)(B, Sq, D)),
            "k_cache": _w((lambda *s: _rng.normal(s) * 0.05)(B, H, Sk, Dh)),
            "v_cache": _w((lambda *s: _rng.normal(s) * 0.05)(B, H, Sk, Dh)),
            "wq": _w((lambda *s: _rng.normal(s) * 0.05)(D, H * Dh) * (D ** -0.5)),
            "wo": _w((lambda *s: _rng.normal(s) * 0.05)(H * Dh, D) * ((H * Dh) ** -0.5)),
        }
    _A_in = _A_setup()

    def _B_setup():
        B, H, Sq, Sk, D, M = 2, 32, 1, 8192, 128, 512
        Dc = 4 * D
        return {
            "x": _w((lambda *s: _rng.normal(s) * 0.05)(B, Sq, M)),
            "c_kv": _w((lambda *s: _rng.normal(s) * 0.05)(B, Sk, Dc)),
            "w_q": _w((lambda *s: _rng.normal(s) * 0.05)(M, H, D) * (M ** -0.5)),
            "w_uk": _w((lambda *s: _rng.normal(s) * 0.05)(Dc, H, D) * (Dc ** -0.5)),
            "w_uv": _w((lambda *s: _rng.normal(s) * 0.05)(Dc, H, D) * (Dc ** -0.5)),
            "w_o": _w((lambda *s: _rng.normal(s) * 0.05)(H, D, M) * ((H * D) ** -0.5)),
        }
    _B_in = _B_setup()

    return {
        "A_x": _A_in["x"],
        "A_k_cache": _A_in["k_cache"],
        "A_v_cache": _A_in["v_cache"],
        "A_wq": _A_in["wq"],
        "A_wo": _A_in["wo"],
        "B_x": _B_in["x"],
        "B_c_kv": _B_in["c_kv"],
        "B_w_q": _B_in["w_q"],
        "B_w_uk": _B_in["w_uk"],
        "B_w_uv": _B_in["w_uv"],
        "B_w_o": _B_in["w_o"],
        "gate_w": _w((lambda *s: _rng.normal(s) * 0.05)(512)),
    }

def reference(A_x, A_k_cache, A_v_cache, A_wq, A_wo, B_x, B_c_kv, B_w_q, B_w_uk, B_w_uv, B_w_o, gate_w):
    def _A_ref(x, k_cache, v_cache, wq, wo):
        B, Sq, D = x.shape
        H, Dh = 32, 128
        q = (lambda x, *d: x.transpose(*d))((x @ wq).reshape(B, Sq, H, Dh), 0, 2, 1, 3)
        scores = jnp.einsum("bhqd,bhkd->bhqk", q, k_cache) * (Dh ** -0.5)
        p = _softmax(scores, axis=-1)
        o = jnp.einsum("bhqk,bhkd->bhqd", p, v_cache)
        return (lambda x, *d: x.transpose(*d))(o, 0, 2, 1, 3).reshape(B, Sq, H * Dh) @ wo

    def _B_ref(x, c_kv, w_q, w_uk, w_uv, w_o):
        B, Sq, M = x.shape[0], x.shape[1], x.shape[2]
        Sk = c_kv.shape[1]
        H, D = w_q.shape[1], w_q.shape[2]
        q = jnp.einsum("bqm,mhd->bhqd", x, w_q)
        k = jnp.einsum("bkc,chd->bhkd", c_kv, w_uk)
        v = jnp.einsum("bkc,chd->bhkd", c_kv, w_uv)
        scores = jnp.einsum("bhqd,bhkd->bhqk", q, k) * (D ** -0.5)
        off = Sk - Sq
        qi = jnp.arange(Sq)[:, None]
        kj = jnp.arange(Sk)[None, :]
        cmask = kj <= (qi + off)
        scores = jnp.where(cmask[None, None], scores, -1e9)
        p = _softmax(scores, axis=-1)
        ctx = jnp.einsum("bhqk,bhkd->bhqd", p, v)
        return jnp.einsum("bhqd,hdm->bqm", ctx, w_o)

    x = A_x
    g = _sigmoid((x * gate_w).sum(-1, keepdims=True))
    a = _A_ref(x, A_k_cache, A_v_cache, A_wq, A_wo)
    b = _B_ref(x, B_c_kv, B_w_q, B_w_uk, B_w_uv, B_w_o)
    return g * a + (1 - g) * b
```

```python
import jax
import jax.numpy as jnp
import jax.experimental.pallas as pl
import jax.experimental.pallas.tpu as pltpu

_B, _H, _SK, _DH, _D, _DC = 2, 32, 8192, 128, 512, 512

_NR = 64
_G = 4
_NU = 4
_SHIFT = 1
_LAG = 13
_E1 = 5
_NBAL = 0
_SPLIT = True
_SCOPES = False

_f32 = jnp.float32
_bf16 = jnp.bfloat16


def _dot(a, b):
    return jnp.dot(a, b, preferred_element_type=_f32)


def _dot_t(a, b):
    return jax.lax.dot_general(a, b, (((1,), (1,)), ((), ())), preferred_element_type=_f32)


def _unpack_pair(blk):
    lo = pltpu.bitcast(blk << 16, _f32).astype(_bf16)
    hi = pltpu.bitcast(blk & jnp.int32(-65536), _f32).astype(_bf16)
    return lo, hi


def _loop(lo, hi, fn):
    def body(i, carry):
        fn(i)
        return carry
    jax.lax.fori_loop(lo, hi, body, 0)


def _kernel(x_hbm, gw_hbm,
            k_hbm, v_hbm, wq_hbm, wo_hbm, ckv_hbm, bwq_hbm, bwuk_hbm, bwuv_hbm, bwo_hbm,
            out_hbm,
            kv_buf, wq_v, wob_v, ckv_v, bwq_v, bwuk_v, bwuv_v,
            qa_s, qb_s, qlat_s, o_s, ctx_s, m_s, l_s, acc_s,
            x_ref, gw_ref, out_v, w32, out_sem):
    out_copy = pltpu.make_async_copy(out_v, out_hbm, out_sem)

    def body(kv_sem, w_sem, c_sem, e_sem, x_sem):
        def start(src, dst, sem, prio):
            pltpu.make_async_copy(src, dst, sem).start(priority=prio)

        def wait_all(dst, sem, name=None):
            if _SCOPES and name:
                with jax.named_scope(name):
                    pltpu.make_async_copy(dst, dst, sem).wait()
            else:
                pltpu.make_async_copy(dst, dst, sem).wait()

        def run(r, rows):
            return pl.ds(pl.multiple_of(r * rows, rows), rows)

        def w_round(r):
            rows = run(r, 64)
            qr, qc = run(r >> 2, 8), run(r & 3, 1024)
            for j in (pl.ds(0, 2), pl.ds(2, 2)):
                start(bwuk_hbm.at[j, rows], bwuk_v.at[j, rows], w_sem.at[2], 0)
                start(bwuv_hbm.at[j, rows], bwuv_v.at[j, rows], w_sem.at[3], 1)
            for j in (pl.ds(0, 2), pl.ds(2, 2)):
                start(bwq_hbm.at[j, rows], bwq_v.at[j, rows], w_sem.at[1], 0)
                start(wq_hbm.at[j, qr, qc], wq_v.at[j, qr, qc], w_sem.at[0], 1)

        RU = _NR // _NU

        def c_round(r):
            u = r >> 4
            src, dst = run(r, 16), run(r & (RU - 1), 16)
            for j in range(0, 8, 2):
                for b in range(_B):
                    start(ckv_hbm.at[b, pl.ds(j, 2), src], ckv_v.at[u, b, pl.ds(j, 2), dst], c_sem.at[u], b)

        def pair_of(i):
            return (i + _SHIFT) & (_B * _H - 1)

        def kv_round(g, r):
            slot = g & 1
            rows = run(r, 64)
            for j in range(_G):
                bh = pair_of(g * _G + j)
                for t, src in enumerate((k_hbm, v_hbm)):
                    start(src.at[bh, :, rows], kv_buf.at[slot, t, j, :, rows], kv_sem.at[slot], t)

        def e_start(t, j, r, sem, prio):
            rows = run(r, 16)
            start((wo_hbm, bwo_hbm)[t].at[pl.ds(j, 2), rows], wob_v.at[t, pl.ds(j, 2), rows], sem, prio)

        def e_round(r):
            for n in range(2):
                for j in (0, 2):
                    for t in range(2):
                        e_start(t, j, 2 * r + n, e_sem.at[r >> 2], t)

        row8 = jax.lax.broadcasted_iota(jnp.int32, (8, _D), 0)
        scale = _DH ** -0.5

        def load_x8():
            xf = x_ref[...].astype(_f32)
            return jnp.where(row8 == 0, xf[0:1], jnp.where(row8 == 1, xf[1:2], 0.0))

        def qa_part(x8, c):
            w = wq_v[:, :, run(c, 4 * _DH)].reshape(_D, 4 * _DH)
            q = _dot(x8, w) * scale
            for j in range(4):
                qa_s[4 * c + j] = q[:, j * _DH:(j + 1) * _DH]

        def to_words(w_v, issue):
            R = 256

            def segment(s):
                issue(s)

                def cp(blk):
                    w32[run(s * 8 + blk, R), :] = pltpu.bitcast(w_v[s, run(blk, 2 * R), :], jnp.int32)
                _loop(0, 8, cp)
            _loop(0, 4, segment)

        def head_pair(i):
            return _unpack_pair(w32[pl.ds(i, _D, stride=_H // 2), :])

        def qb_pair(x8, i):
            lo, hi = head_pair(i)
            qb_s[2 * i] = _dot(x8, lo)
            qb_s[2 * i + 1] = _dot(x8, hi)

        def qlat_pair(i):
            pair = head_pair(i)
            for j in range(2):
                h = 2 * i + j
                ql = _dot_t(qb_s[h].astype(_bf16), pair[j]) * scale
                qlat_s[0, pl.ds(h, 1), :] = ql[0:1, :]
                qlat_s[1, pl.ds(h, 1), :] = ql[1:2, :]

        def b_chunk(u, b, c):
            ck = ckv_v[u, b, pl.ds(4 * c, 4)].reshape(1024, _DC)
            s = _dot_t(qlat_s[b].astype(_bf16), ck)
            m_old = m_s[b]
            m_new = jnp.maximum(m_old, jnp.max(s, axis=-1, keepdims=True))
            p = jnp.exp(s - m_new)
            alpha = jnp.exp(m_old - m_new)
            m_s[b] = m_new
            l_s[b] = alpha * l_s[b] + jnp.sum(p, axis=-1, keepdims=True)
            acc_s[b] = alpha * acc_s[b] + _dot(p.astype(_bf16), ck)

        def ctx_pair(i):
            pair = head_pair(i)
            for j in range(2):
                h = 2 * i + j
                r0 = acc_s[0, pl.ds(h, 1), :]
                r1 = acc_s[1, pl.ds(h, 1), :]
                lhs = jnp.where(row8 == 0, r0, jnp.where(row8 == 1, r1, 0.0))
                ctx_s[h] = _dot(lhs.astype(_bf16), pair[j])

        row8h = jax.lax.broadcasted_iota(jnp.int32, (8, _DH), 0)

        def a_head(i):
            slot, j = (i >> 2) & 1, i & 3
            bh = pair_of(i)
            b, h = bh >> 5, bh & (_H - 1)
            q8 = qa_s[h].astype(_bf16)
            s = _dot_t(q8, kv_buf[slot, 0, j].reshape(_SK, _DH))
            m = jnp.max(s, axis=-1, keepdims=True)
            p = jnp.exp(s - m)
            l = jnp.sum(p, axis=-1, keepdims=True)
            o = _dot(p.astype(_bf16), kv_buf[slot, 1, j].reshape(_SK, _DH)) / l
            o_s[h] = jnp.where(row8h == b, o, o_s[h])

        def out_proj(i, segs, carry):
            res = []
            for t, src_s in enumerate((o_s, ctx_s)):
                acc = carry[t]
                for s in segs:
                    acc = acc + _dot(src_s[8 * s + i].astype(_bf16), wob_v[t, s, run(i, _DH), :])
                res.append(acc)
            return tuple(res)

        w_round(0)
        cx = pltpu.make_async_copy(x_hbm, x_ref, x_sem.at[0])
        cg = pltpu.make_async_copy(gw_hbm, gw_ref, x_sem.at[1])
        cx.start()
        cg.start()
        _loop(1, _NR, w_round)
        o_s[...] = jnp.zeros_like(o_s)
        m_s[...] = jnp.full_like(m_s, -jnp.inf)
        l_s[...] = jnp.zeros_like(l_s)
        acc_s[...] = jnp.zeros_like(acc_s)
        cx.wait()
        cg.wait()
        x8f = load_x8()
        x8 = x8f.astype(_bf16)
        gate = jax.nn.sigmoid(jnp.sum(x8f * gw_ref[...].astype(_f32).reshape(1, _D), axis=-1, keepdims=True))

        def ck_round(r):
            @pl.when(r < _NR)
            def _():
                c_round(r)

            @pl.when(r >= _NR)
            def _():
                kv_round(0, r - _NR)

        r0 = _LAG
        _loop(0, r0, c_round)
        wait_all(wq_v, w_sem.at[0], 'ww')

        def qa_step(c):
            @pl.when(c & 1 == 0)
            def _():
                c_round(r0 + (c >> 1))
            qa_part(x8, c)
        _loop(0, 8, qa_step)
        wait_all(bwq_v, w_sem.at[1])
        to_words(bwq_v, lambda s: c_round(r0 + 4 + s))

        def qb_step(i):
            c_round(r0 + 8 + i)
            qb_pair(x8, i)
        _loop(0, 16, qb_step)
        wait_all(bwuk_v, w_sem.at[2])
        to_words(bwuk_v, lambda s: c_round(r0 + 24 + s))

        def qlat_step(i):
            c_round(r0 + 28 + i)
            qlat_pair(i)
        _loop(0, 16, qlat_step)
        r1 = r0 + 44

        def b_step(t):
            u = t >> 2
            _loop(r1 + 3 * t, r1 + 3 * t + 3, ck_round)

            @pl.when(t & 3 == 0)
            def _():
                wait_all(ckv_v.at[u], c_sem.at[u], 'cw')
            b_chunk(u, t & 1, (t >> 1) & 1)
        _loop(0, 16, b_step)
        acc_s[...] = acc_s[...] / l_s[...]
        r2 = r1 + 48 - _NR

        wait_all(bwuv_v, w_sem.at[3])
        to_words(bwuv_v, lambda s: kv_round(0, r2 + s))

        def ctx_step(i):
            kv_round(0, r2 + 4 + i)
            ctx_pair(i)
        _loop(0, 16, ctx_step)
        _loop(r2 + 20, _NR, lambda r: kv_round(0, r))

        nbh = _B * _H
        RH = _NR // _G

        def a_step(i):
            g, j = i >> 2, i & 3

            @pl.when(i < nbh - _G)
            def _():
                _loop(j * RH, (j + 1) * RH, lambda r: kv_round(g + 1, r))

            @pl.when(i >= nbh - _G)
            def _():
                _loop(jnp.where(j == 0, 0, _LAG + _E1 * (j - 1)), _LAG + _E1 * j, e_round)

            @pl.when(j == 0)
            def _():
                wait_all(kv_buf.at[g & 1], kv_sem.at[g & 1], 'kvw')
            a_head(i)
        _loop(0, nbh, a_step)

        _loop(_LAG + _E1 * (_G - 1), 28, e_round)
        if _SPLIT:
            tail = [(t, j, r, 7 + j // 2) for j in (0, 2) for r in range(56, 64) for t in range(2)]
        else:
            tail = [(t, j, r, 7 + j // 2) for r in range(56, 64) for j in (0, 2) for t in range(2)]
        for n, (t, j, r, e) in enumerate(tail):
            e_start(t, j, r, e_sem.at[e], t if n < len(tail) - 2 * _NBAL else 0)

        def e_step(i, carry):
            wait_all(wob_v.at[:, :, run(i, _DH)], e_sem.at[i], 'ew')
            return out_proj(i, range(4), carry)
        zero = jnp.zeros((8, _D), _f32)
        carry = jax.lax.fori_loop(0, 7, e_step, (zero, zero))
        for j in (0, 2):
            wait_all(wob_v.at[:, pl.ds(j, 2), run(7, _DH)], e_sem.at[7 + j // 2], 'ew')
            carry = out_proj(7, (j, j + 1), carry)
        res = gate * carry[0] + (1.0 - gate) * carry[1]
        out_v[...] = res[0:2, :].astype(_bf16)
        out_copy.start()

    dma = pltpu.SemaphoreType.DMA
    pl.run_scoped(body, dma((2,)), dma((4,)), dma((_NU,)), dma((9,)), dma((2,)))
    out_copy.wait()


@jax.jit
def pallas_gated_mix__mha_block_cached__compressed_kv_cla__decode_kernel(
    A_x: jax.Array,
    A_k_cache: jax.Array,
    A_v_cache: jax.Array,
    A_wq: jax.Array,
    A_wo: jax.Array,
    B_x: jax.Array,
    B_c_kv: jax.Array,
    B_w_q: jax.Array,
    B_w_uk: jax.Array,
    B_w_uv: jax.Array,
    B_w_o: jax.Array,
    gate_w: jax.Array,
):
    del B_x
    k4 = A_k_cache.reshape(_B * _H, 2, _SK // 2, _DH)
    v4 = A_v_cache.reshape(_B * _H, 2, _SK // 2, _DH)
    wq = A_wq.reshape(4, _D // 4, _H * _DH)
    wo = A_wo.reshape(4, _H * _DH // 4, _D)
    ckv = B_c_kv.reshape(_B, 8, _SK // 8, _DC)
    bwq = B_w_q.reshape(4, _D * _H // 4, _DH)
    bwuk = B_w_uk.reshape(4, _DC * _H // 4, _DH)
    bwuv = B_w_uv.reshape(4, _DC * _H // 4, _DH)
    bwo = B_w_o.reshape(4, _H * _DH // 4, _D)
    x2 = A_x.reshape(_B, _D)

    hbm = pl.BlockSpec(memory_space=pl.ANY)
    V = pltpu.VMEM
    scratch = [
        V((2, 2, _G, 2, _SK // 2, _DH), _bf16),
        V(wq.shape, _bf16),
        V((2,) + wo.shape, _bf16),
        V((_NU, _B, 8, _SK // 8 // _NU, _DC), _bf16),
        V(bwq.shape, _bf16),
        V(bwuk.shape, _bf16),
        V(bwuv.shape, _bf16),
        V((_H, 8, _DH), _f32),
        V((_H, 8, _DH), _f32),
        V((_B, _H, _DC), _f32),
        V((_H, 8, _DH), _f32),
        V((_H, 8, _DH), _f32),
        V((_B, _H, 1), _f32),
        V((_B, _H, 1), _f32),
        V((_B, _H, _DC), _f32),
        V((_B, _D), _bf16),
        V((_D,), _bf16),
        V((_B, _D), _bf16),
        V((_D * _H // 2, _DH), jnp.int32),
        pltpu.SemaphoreType.DMA(()),
    ]
    out = pl.pallas_call(
        _kernel,
        out_shape=jax.ShapeDtypeStruct((_B, _D), _bf16),
        in_specs=[hbm] * 11,
        out_specs=hbm,
        scratch_shapes=scratch,
        compiler_params=pltpu.CompilerParams(vmem_limit_bytes=100 * 1024 * 1024, disable_bounds_checks=True),
    )(x2, gate_w, k4, v4, wq, wo, ckv, bwq, bwuk, bwuv, bwo)
    return out.reshape(_B, 1, _D)
```

```python
import jax
import jax.numpy as jnp
import jax.experimental.pallas as pl
import jax.experimental.pallas.tpu as pltpu

_B, _H, _SK, _DH, _D, _DC = 2, 32, 8192, 128, 512, 512

_NR = 64
_G = 4
_NU = 4
_FIRST = 1
_V_AHEAD = 7
_QUEUED = 13
_E_STEP = 5

_f32 = jnp.float32
_bf16 = jnp.bfloat16


def _dot(a, b):
    return jnp.dot(a, b, preferred_element_type=_f32)


def _dot_t(a, b):
    return jax.lax.dot_general(a, b, (((1,), (1,)), ((), ())), preferred_element_type=_f32)


def _loop(lo, hi, fn):
    def body(i, carry):
        fn(i)
        return carry
    jax.lax.fori_loop(lo, hi, body, 0)


def _run(i, size):
    return pl.ds(pl.multiple_of(i * size, size), size)


def _start(src, dst, sem, queue):
    pltpu.make_async_copy(src, dst, sem).start(priority=queue)


def _wait_all(dst, sem):
    pltpu.make_async_copy(dst, dst, sem).wait()


def _kernel(x_hbm, gw_hbm, k_hbm, v_hbm, wq_hbm, wo_hbm, ckv_hbm, bwq_hbm, bwuk_hbm, bwuv_hbm, bwo_hbm,
            out_hbm,
            kv_v, wq_v, wob_v, ckv_v, bwq_v, bwuk_v, bwuv_v, x_v, gw_v, out_v,
            w32, qa_s, qb_s, qlat_s, o_s, ctx_s, m_s, l_s, acc_s, out_sem):
    out_copy = pltpu.make_async_copy(out_v, out_hbm, out_sem)

    def body(x_sem, w_sem, c_sem, kv_sem, e_sem):
        def w_round(r):
            rows = _run(r, 64)
            for j in (pl.ds(0, 2), pl.ds(2, 2)):
                _start(bwuv_hbm.at[j, rows], bwuv_v.at[j, rows], w_sem.at[3], 0)
                _start(bwq_hbm.at[j, rows], bwq_v.at[j, rows], w_sem.at[1], 1)
            wq_rows, wq_cols = _run(r >> 2, 8), _run(r & 3, 1024)
            for j in (pl.ds(0, 2), pl.ds(2, 2)):
                _start(bwuk_hbm.at[j, rows], bwuk_v.at[j, rows], w_sem.at[2], 0)
                _start(wq_hbm.at[j, wq_rows, wq_cols], wq_v.at[j, wq_rows, wq_cols], w_sem.at[0], 1)

        def c_round(r):
            u = r >> 4
            src, dst = _run(r, 16), _run(r & 15, 16)
            for j in range(0, 8, 2):
                for b in range(_B):
                    _start(ckv_hbm.at[b, pl.ds(j, 2), src], ckv_v.at[u, b, pl.ds(j, 2), dst], c_sem.at[u], b)

        def pair_of(i):
            return (i + _FIRST) & (_B * _H - 1)

        def kv_round(g, r):
            slot = g & 1
            rows = _run(r, 64), _run((r + _V_AHEAD) & (_NR - 1), 64)
            for n in range(_G):
                for t, (src, j) in enumerate(((k_hbm, n), (v_hbm, _G - 1 - n))):
                    _start(src.at[pair_of(g * _G + j), :, rows[t]], kv_v.at[slot, t, j, :, rows[t]],
                           kv_sem.at[slot], t)

        def e_piece(t, j, r, sem):
            src = _run((r + 16 * j) & (_NR - 1), 16)
            _start((wo_hbm, bwo_hbm)[t].at[pl.ds(j, 2), src], wob_v.at[t, pl.ds(j, 2), _run(r, 16)], sem, t)

        def e_round(r):
            for n in range(2):
                for j in (0, 2):
                    for t in range(2):
                        e_piece(t, j, 2 * r + n, e_sem.at[r >> 2])

        row8 = jax.lax.broadcasted_iota(jnp.int32, (8, _D), 0)
        row8h = jax.lax.broadcasted_iota(jnp.int32, (8, _DH), 0)
        scale = _DH ** -0.5

        def two_rows(r0, r1):
            return jnp.where(row8 == 0, r0, jnp.where(row8 == 1, r1, 0.0))

        def qa_part(x8, c):
            q = _dot(x8, wq_v[:, :, _run(c, 4 * _DH)].reshape(_D, 4 * _DH)) * scale
            for j in range(4):
                qa_s[4 * c + j] = q[:, j * _DH:(j + 1) * _DH]

        def to_words(w_v, issue):
            def segment(s):
                issue(s)

                def part(n):
                    w32[_run(s * 8 + n, 256), :] = pltpu.bitcast(w_v[s, _run(n, 512), :], jnp.int32)
                _loop(0, 8, part)
            _loop(0, 4, segment)

        def head_pair(i):
            words = w32[pl.ds(i, _D, stride=_H // 2), :]
            return (pltpu.bitcast(words << 16, _f32).astype(_bf16),
                    pltpu.bitcast(words & jnp.int32(-65536), _f32).astype(_bf16))

        def qb_pair(x8, i):
            for j, w in enumerate(head_pair(i)):
                qb_s[2 * i + j] = _dot(x8, w)

        def qlat_pair(i):
            for j, w in enumerate(head_pair(i)):
                h = 2 * i + j
                ql = _dot_t(qb_s[h].astype(_bf16), w) * scale
                qlat_s[0, pl.ds(h, 1), :] = ql[0:1, :]
                qlat_s[1, pl.ds(h, 1), :] = ql[1:2, :]

        def b_chunk(u, b, c):
            ck = ckv_v[u, b, pl.ds(4 * c, 4)].reshape(1024, _DC)
            s = _dot_t(qlat_s[b].astype(_bf16), ck)
            m_old = m_s[b]
            m_new = jnp.maximum(m_old, jnp.max(s, axis=-1, keepdims=True))
            p = jnp.exp(s - m_new)
            alpha = jnp.exp(m_old - m_new)
            m_s[b] = m_new
            l_s[b] = alpha * l_s[b] + jnp.sum(p, axis=-1, keepdims=True)
            acc_s[b] = alpha * acc_s[b] + _dot(p.astype(_bf16), ck)

        def ctx_pair(i):
            for j, w in enumerate(head_pair(i)):
                h = 2 * i + j
                lhs = two_rows(acc_s[0, pl.ds(h, 1), :], acc_s[1, pl.ds(h, 1), :])
                ctx_s[h] = _dot(lhs.astype(_bf16), w)

        def a_head(i):
            slot, j = (i >> 2) & 1, i & 3
            bh = pair_of(i)
            b, h = bh >> 5, bh & (_H - 1)
            q8 = qa_s[h].astype(_bf16)
            s = _dot_t(q8, kv_v[slot, 0, j].reshape(_SK, _DH))
            m = jnp.max(s, axis=-1, keepdims=True)
            p = jnp.exp(s - m)
            l = jnp.sum(p, axis=-1, keepdims=True)
            o = _dot(p.astype(_bf16), kv_v[slot, 1, j].reshape(_SK, _DH)) / l
            o_s[h] = jnp.where(row8h == b, o, o_s[h])

        def out_proj(i, segments, carry):
            res = []
            for t, src_s in enumerate((o_s, ctx_s)):
                acc = carry[t]
                for s in segments:
                    h = 8 * s + ((i + 2 * (s & 2)) & 7)
                    acc = acc + _dot(src_s[h].astype(_bf16), wob_v[t, s, _run(i, _DH), :])
                res.append(acc)
            return tuple(res)

        w_round(0)
        x_copy = pltpu.make_async_copy(x_hbm, x_v, x_sem.at[0])
        gw_copy = pltpu.make_async_copy(gw_hbm, gw_v, x_sem.at[1])
        x_copy.start()
        gw_copy.start()
        _loop(1, _NR, w_round)
        o_s[...] = jnp.zeros_like(o_s)
        m_s[...] = jnp.full_like(m_s, -jnp.inf)
        l_s[...] = jnp.zeros_like(l_s)
        acc_s[...] = jnp.zeros_like(acc_s)
        x_copy.wait()
        gw_copy.wait()
        xf = x_v[...].astype(_f32)
        x8f = two_rows(xf[0:1], xf[1:2])
        x8 = x8f.astype(_bf16)
        gate = jax.nn.sigmoid(jnp.sum(x8f * gw_v[...].astype(_f32).reshape(1, _D), axis=-1, keepdims=True))

        _loop(0, _QUEUED, c_round)
        _wait_all(wq_v, w_sem.at[0])

        def qa_step(c):
            @pl.when(c & 1 == 0)
            def _():
                c_round(_QUEUED + (c >> 1))
            qa_part(x8, c)
        _loop(0, 8, qa_step)
        _wait_all(bwq_v, w_sem.at[1])
        to_words(bwq_v, lambda s: c_round(_QUEUED + 4 + s))

        def qb_step(i):
            c_round(_QUEUED + 8 + i)
            qb_pair(x8, i)
        _loop(0, 16, qb_step)
        _wait_all(bwuk_v, w_sem.at[2])
        to_words(bwuk_v, lambda s: c_round(_QUEUED + 24 + s))

        def qlat_step(i):
            c_round(_QUEUED + 28 + i)
            qlat_pair(i)
        _loop(0, 16, qlat_step)

        r_b = _QUEUED + 44

        def ck_round(r):
            @pl.when(r < _NR)
            def _():
                c_round(r)

            @pl.when(r >= _NR)
            def _():
                kv_round(0, r - _NR)

        def b_step(t):
            u = t >> 2
            _loop(r_b + 3 * t, r_b + 3 * t + 3, ck_round)

            @pl.when(t & 3 == 0)
            def _():
                _wait_all(ckv_v.at[u], c_sem.at[u])
            b_chunk(u, t & 1, (t >> 1) & 1)
        _loop(0, 16, b_step)
        acc_s[...] = acc_s[...] / l_s[...]

        r_ctx = r_b + 48 - _NR
        _wait_all(bwuv_v, w_sem.at[3])
        to_words(bwuv_v, lambda s: kv_round(0, r_ctx + s))

        def ctx_step(i):
            kv_round(0, r_ctx + 4 + i)
            ctx_pair(i)
        _loop(0, 16, ctx_step)
        _loop(r_ctx + 20, _NR, lambda r: kv_round(0, r))

        def a_step(i):
            g, j = i >> 2, i & 3

            @pl.when(i < _B * _H - _G)
            def _():
                _loop(j * (_NR // _G), (j + 1) * (_NR // _G), lambda r: kv_round(g + 1, r))

            @pl.when(i >= _B * _H - _G)
            def _():
                _loop(jnp.where(j == 0, 0, _QUEUED + _E_STEP * (j - 1)), _QUEUED + _E_STEP * j, e_round)

            @pl.when(j == 0)
            def _():
                _wait_all(kv_v.at[g & 1], kv_sem.at[g & 1])
            a_head(i)
        _loop(0, _B * _H, a_step)

        assert _QUEUED + _E_STEP * (_G - 1) == 28
        for j in (0, 2):
            for r in range(56, 64):
                for t in range(2):
                    e_piece(t, j, r, e_sem.at[7 + j // 2])

        def e_step(i, carry):
            _wait_all(wob_v.at[:, :, _run(i, _DH)], e_sem.at[i])
            return out_proj(i, range(4), carry)
        zero = jnp.zeros((8, _D), _f32)
        carry = jax.lax.fori_loop(0, 7, e_step, (zero, zero))
        for j in (0, 2):
            _wait_all(wob_v.at[:, pl.ds(j, 2), _run(7, _DH)], e_sem.at[7 + j // 2])
            carry = out_proj(7, (j, j + 1), carry)
        res = gate * carry[0] + (1.0 - gate) * carry[1]
        out_v[...] = res[0:2, :].astype(_bf16)
        out_copy.start()

    dma = pltpu.SemaphoreType.DMA
    pl.run_scoped(body, dma((2,)), dma((4,)), dma((_NU,)), dma((2,)), dma((9,)))
    out_copy.wait()


@jax.jit
def pallas_gated_mix__mha_block_cached__compressed_kv_cla__decode_kernel(
    A_x: jax.Array,
    A_k_cache: jax.Array,
    A_v_cache: jax.Array,
    A_wq: jax.Array,
    A_wo: jax.Array,
    B_x: jax.Array,
    B_c_kv: jax.Array,
    B_w_q: jax.Array,
    B_w_uk: jax.Array,
    B_w_uv: jax.Array,
    B_w_o: jax.Array,
    gate_w: jax.Array,
):
    del B_x
    k = A_k_cache.reshape(_B * _H, 2, _SK // 2, _DH)
    v = A_v_cache.reshape(_B * _H, 2, _SK // 2, _DH)
    wq = A_wq.reshape(4, _D // 4, _H * _DH)
    wo = A_wo.reshape(4, _H * _DH // 4, _D)
    ckv = B_c_kv.reshape(_B, 8, _SK // 8, _DC)
    bwq = B_w_q.reshape(4, _D * _H // 4, _DH)
    bwuk = B_w_uk.reshape(4, _DC * _H // 4, _DH)
    bwuv = B_w_uv.reshape(4, _DC * _H // 4, _DH)
    bwo = B_w_o.reshape(4, _H * _DH // 4, _D)
    x = A_x.reshape(_B, _D)

    hbm = pl.BlockSpec(memory_space=pl.ANY)
    V = pltpu.VMEM
    scratch = [
        V((2, 2, _G, 2, _SK // 2, _DH), _bf16),
        V(wq.shape, _bf16),
        V((2,) + wo.shape, _bf16),
        V((_NU, _B, 8, _SK // 8 // _NU, _DC), _bf16),
        V(bwq.shape, _bf16),
        V(bwuk.shape, _bf16),
        V(bwuv.shape, _bf16),
        V((_B, _D), _bf16),
        V((_D,), _bf16),
        V((_B, _D), _bf16),
        V((_D * _H // 2, _DH), jnp.int32),
        V((_H, 8, _DH), _f32),
        V((_H, 8, _DH), _f32),
        V((_B, _H, _DC), _f32),
        V((_H, 8, _DH), _f32),
        V((_H, 8, _DH), _f32),
        V((_B, _H, 1), _f32),
        V((_B, _H, 1), _f32),
        V((_B, _H, _DC), _f32),
        pltpu.SemaphoreType.DMA(()),
    ]
    out = pl.pallas_call(
        _kernel,
        out_shape=jax.ShapeDtypeStruct((_B, _D), _bf16),
        in_specs=[hbm] * 11,
        out_specs=hbm,
        scratch_shapes=scratch,
        compiler_params=pltpu.CompilerParams(vmem_limit_bytes=100 * 1024 * 1024, disable_bounds_checks=True),
    )(x, gate_w, k, v, wq, wo, ckv, bwq, bwuk, bwuv, bwo)
    return out.reshape(_B, 1, _D)
```
